```python
import os as _os
_os.environ.setdefault("JAX_PLATFORMS", "cpu")
import jax
import jax.numpy as jnp

def _softmax(x, axis=-1):
    return jax.nn.softmax(x, axis=axis)
def _gelu(x):
    return jax.nn.gelu(x, approximate=True)
def _silu(x):
    return jax.nn.silu(x)
def _sigmoid(x):
    return jax.nn.sigmoid(x)
def _layernorm(x, axis=-1, eps=1e-5):
    m = jnp.mean(x, axis=axis, keepdims=True)
    v = jnp.var(x, axis=axis, keepdims=True)
    return (x - m) / jnp.sqrt(v + eps)
def _scatter_add(tgt, idx, src, axis=0):
    return tgt.at[idx].add(src)
def _segment_sum(src, seg, n):
    return jax.ops.segment_sum(src, seg, n)
class _Rng:
    def __init__(self, key):
        self._k = key
    def _next(self):
        self._k, sub = jax.random.split(self._k)
        return sub
    def normal(self, shape):
        return jax.random.normal(self._next(), shape, dtype=jnp.bfloat16)
    def randint(self, lo, hi, shape):
        return jax.random.randint(self._next(), shape, lo, hi, dtype=jnp.int32)
    def uniform(self, shape, lo=0.0, hi=1.0):
        return jax.random.uniform(self._next(), shape, jnp.bfloat16, lo, hi)
    def permutation(self, n):
        return jax.random.permutation(self._next(), n)


kernel_name = 'standalone__gqa_block_cached__near_ridge'

def setup_inputs():
    _rng = _Rng(jax.random.key(int.from_bytes(__import__("os").urandom(4), "little")))
    _w = (lambda a: (lambda t: t.astype(jnp.bfloat16) if jnp.issubdtype(t.dtype, jnp.floating) else t)(jnp.asarray(a)))
    B, Sq, D = 16, 96, 576
    Hq, Hkv, Sk, Dh = 32, 16, 512, 128
    assert Hq % Hkv == 0, (Hq, Hkv)
    return {
        "x": _w((lambda *s: _rng.normal(s) * 0.2)(B, Sq, D)),
        "k_cache": _w((lambda *s: _rng.normal(s) * 3.2)(B, Hkv, Sk, Dh)),
        "v_cache": _w((lambda *s: _rng.normal(s) * 0.05)(B, Hkv, Sk, Dh)),
        "wq": _w((lambda *s: _rng.normal(s) * 0.2)(D, Hq * Dh) * (D ** -0.5)),
        "wo": _w((lambda *s: _rng.normal(s) * 0.05)(Hq * Dh, D) * ((Hq * Dh) ** -0.5)),
    }

def reference(x, k_cache, v_cache, wq, wo):
    B, Sq, D = x.shape
    Hq, Dh = 32, 128
    Hkv = k_cache.shape[1]
    rep = Hq // Hkv
    q = (lambda x, *d: x.transpose(*d))((x @ wq).reshape(B, Sq, Hq, Dh), 0, 2, 1, 3)
    k = jnp.repeat(k_cache, rep, axis=1)
    v = jnp.repeat(v_cache, rep, axis=1)
    scores = jnp.einsum("bhqd,bhkd->bhqk", q, k) * (Dh ** -0.5)
    p = _softmax(scores, axis=-1)
    o = jnp.einsum("bhqk,bhkd->bhqd", p, v)
    return (lambda x, *d: x.transpose(*d))(o, 0, 2, 1, 3).reshape(B, Sq, Hq * Dh) @ wo
```

```python
import functools, math
import jax
import jax.numpy as jnp
import jax.experimental.pallas as pl
import jax.experimental.pallas.tpu as pltpu

B, SQ, D = 16, 96, 576
HQ, HKV, SK, DH = 32, 16, 512, 128
REP = HQ // HKV
M = B * SQ
GB = 4
NG = B // GB
GM = GB * SQ
NT_DIMS = (((1,), (1,)), ((), ()))
bf = jnp.bfloat16
f32 = jnp.float32


def impl(x, k_cache, v_cache, wq, wo, CW=512, recip="approx", XR=384, xstages=(1, 2, 1), scopes=False, vmem_mb=120):
    x2 = x.reshape(M, D)
    wot = wo.T
    c = (DH ** -0.5) * math.log2(math.e)
    NC = (HQ * DH) // CW
    HPC = CW // DH
    NX = M // XR
    assert sum(xstages) == NX
    import contextlib
    scope = jax.named_scope if scopes else (lambda n: contextlib.nullcontext())

    def kernel(x_hbm, k_hbm, v_hbm, wq_hbm, wot_hbm, out_hbm,
               x_v, wq_v, wot_v, k_v, v_v, q_v, o_v, y_v,
               x_sem, wq_sem, wot_sem, kv_sem, out_sem):
        def x_cp(i):
            r0 = i * XR if isinstance(i, int) else pl.multiple_of(i * XR, XR)
            return pltpu.make_async_copy(x_hbm.at[pl.ds(r0, XR)], x_v.at[pl.ds(r0, XR)], x_sem.at[i])

        def wq_cp(ci):
            c0 = ci * CW if isinstance(ci, int) else pl.multiple_of(ci * CW, CW)
            return pltpu.make_async_copy(wq_hbm.at[:, pl.ds(c0, CW)], wq_v.at[ci], wq_sem.at[ci])

        def wot_cp():
            return pltpu.make_async_copy(wot_hbm, wot_v, wot_sem.at[0])

        def k_cp(g):
            return pltpu.make_async_copy(k_hbm.at[pl.ds(g * GB, GB)], k_v.at[pl.ds(g * GB, GB)], kv_sem.at[2 * g])

        def v_cp(g):
            return pltpu.make_async_copy(v_hbm.at[pl.ds(g * GB, GB)], v_v.at[pl.ds(g * GB, GB)], kv_sem.at[2 * g + 1])

        def out_cp(g):
            return pltpu.make_async_copy(y_v.at[g], out_hbm.at[pl.ds(g * GM, GM)], out_sem.at[g])

        x_cp(0).start()
        wq_cp(0).start()

        def start_x(i, carry):
            x_cp(i).start(priority=1)
            return carry

        def start_wq(ci, carry):
            wq_cp(ci).start(priority=1)
            return carry

        def start_kv(g, carry):
            k_cp(g).start(priority=1)
            v_cp(g).start(priority=1)
            return carry

        jax.lax.fori_loop(1, NX, start_x, 0)
        jax.lax.fori_loop(1, NC, start_wq, 0)
        k_cp(0).start(priority=1)
        v_cp(0).start(priority=1)
        wot_cp().start(priority=1)
        jax.lax.fori_loop(1, NG, start_kv, 0)

        def qproj(ci, r0, nr):
            q = jnp.dot(x_v[pl.ds(r0, nr), :], wq_v[ci], preferred_element_type=f32)
            q_v[ci, pl.ds(r0, nr), :] = (q * c).astype(bf)

        i0 = 0
        for si, nx in enumerate(xstages):
            with scope(f"wait_x{si}"):
                for i in range(i0, i0 + nx):
                    x_cp(i).wait()
                if si == 0:
                    wq_cp(0).wait()
            with scope(f"qp0_{si}"):
                qproj(0, i0 * XR, nx * XR)
            i0 += nx

        def p1_body(ci, carry):
            with scope("wait_wq"):
                wq_cp(ci).wait()
            with scope("qp"):
                qproj(ci, 0, M)
            return carry

        jax.lax.fori_loop(1, NC, p1_body, 0)
        wot_cp().wait()

        def p2_body(g, carry):
            with scope("wait_kv"):
                k_cp(g).wait()
                v_cp(g).wait()
            row0 = pl.multiple_of(g * GM, GM)

            def qk(u):
                bb, h = u
                ci, off = (REP * h) // HPC, ((REP * h) % HPC) * DH
                rows = pl.ds(row0 + bb * SQ, SQ)
                qq = jnp.concatenate(
                    [q_v[ci, rows, off + r * DH: off + (r + 1) * DH] for r in range(REP)], axis=0)
                return jax.lax.dot_general(qq, k_v[g * GB + bb, h], NT_DIMS, preferred_element_type=f32)

            def finish(u, s):
                bb, h = u
                m = jnp.max(s, axis=-1, keepdims=True)
                p = jnp.exp2(s - m)
                l = jnp.sum(p, axis=-1, keepdims=True)
                o = jnp.dot(p.astype(bf), v_v[g * GB + bb, h], preferred_element_type=f32)
                if recip == "approx":
                    r = pl.reciprocal(l, approx=True)
                elif recip == "newton":
                    r = pl.reciprocal(l, approx=True)
                    r = r * (2.0 - l * r)
                else:
                    r = pl.reciprocal(l, approx=False)
                o = (o * r).astype(bf)
                for r_ in range(REP):
                    col = (REP * h + r_) * DH
                    o_v[bb * SQ:(bb + 1) * SQ, col:col + DH] = o[r_ * SQ:(r_ + 1) * SQ]

            def oproj(t):
                ot = o_v[t * 128:(t + 1) * 128, :]
                for dc in range(5):
                    lo, hi = dc * 128, min((dc + 1) * 128, D)
                    r = jax.lax.dot_general(wot_v[lo:hi, :], ot, NT_DIMS, preferred_element_type=f32)
                    y_v[g, t * 128:(t + 1) * 128, lo:hi] = r.T.astype(bf)

            units = [(bb, h) for bb in range(GB) for h in range(HKV)]
            s = qk(units[0])
            for i, u in enumerate(units):
                s_next = qk(units[i + 1]) if i + 1 < len(units) else None
                finish(u, s)
                s = s_next
                if u == (2, 0):
                    oproj(0)
                if u == (3, 0):
                    oproj(1)
            oproj(2)
            out_cp(g).start()
            return carry

        with scope("p2"):
            jax.lax.fori_loop(0, NG, p2_body, 0)
        with scope("wait_out"):
            for g in range(NG):
                out_cp(g).wait()

    hbm = pl.BlockSpec(memory_space=pl.ANY)
    out = pl.pallas_call(
        kernel,
        in_specs=[hbm] * 5,
        out_specs=hbm,
        out_shape=jax.ShapeDtypeStruct((M, D), x.dtype),
        scratch_shapes=[
            pltpu.VMEM((M, D), bf),
            pltpu.VMEM((NC, D, CW), bf),
            pltpu.VMEM((D, HQ * DH), bf),
            pltpu.VMEM((B, HKV, SK, DH), bf),
            pltpu.VMEM((B, HKV, SK, DH), bf),
            pltpu.VMEM((NC, M, CW), bf),
            pltpu.VMEM((GM, HQ * DH), bf),
            pltpu.VMEM((NG, GM, D), bf),
            pltpu.SemaphoreType.DMA((NX,)),
            pltpu.SemaphoreType.DMA((NC,)),
            pltpu.SemaphoreType.DMA((1,)),
            pltpu.SemaphoreType.DMA((2 * NG,)),
            pltpu.SemaphoreType.DMA((NG,)),
        ],
        compiler_params=pltpu.CompilerParams(vmem_limit_bytes=vmem_mb * 1024 * 1024),
    )(x2, k_cache, v_cache, wq, wot)
    return out.reshape(B, SQ, D)


@jax.jit
def pallas_standalone__gqa_block_cached__near_ridge_kernel(x, k_cache, v_cache, wq, wo):
    return impl(x, k_cache, v_cache, wq, wo)
```

```python
import math

import jax
import jax.numpy as jnp
import jax.experimental.pallas as pl
import jax.experimental.pallas.tpu as pltpu

B, SQ, D = 16, 96, 576
HQ, HKV, SK, DH = 32, 16, 512, 128
REP = HQ // HKV
M = B * SQ
GB = 4
NG = B // GB
GM = GB * SQ
TT = 128
DF = (D // 128) * 128
XR = 128
NX = M // XR

H0 = 4
HL = 12
NL = 2
HX = 4
HXO = HQ - HX
assert H0 + NL * HL + HX == HQ

STAGES = ((1, 2), (2, 3), (3, 4), (6, 4), (NX, H0))
PIECES = (0, 192, 320, 384)
NP = len(PIECES) - 1
NW = DF // 128
O_LAG = 3
OUT_LAG = 3

NT_DIMS = (((1,), (1,)), ((), ()))
Q_SCALE = (DH ** -0.5) * math.log2(math.e)
bf16 = jnp.bfloat16
f32 = jnp.float32


def _kernel(x_hbm, k_hbm, v_hbm, wq_hbm, wot_hbm, out_hbm,
            x_v, wq0_v, wql_v, wqx_v, wot_v, k_v, v_v, q0_v, ql_v, qx_v, o_v, y_v,
            x_sem, wq0_sem, wql_sem, w_sem, kv_sem, out_sem):
    def aligned(i, n):
        return i if isinstance(i, int) else pl.multiple_of(i, n)

    def x_cp(i):
        rows = pl.ds(aligned(i * XR, XR), XR)
        return pltpu.make_async_copy(x_hbm.at[rows], x_v.at[rows], x_sem.at[i])

    def wq0_cp(h):
        cols = pl.ds(aligned(h * DH, DH), DH)
        return pltpu.make_async_copy(wq_hbm.at[:, cols], wq0_v.at[:, cols], wq0_sem.at[h])

    def wql_cp(ci):
        cols = pl.ds(aligned((H0 + ci * HL) * DH, DH), HL * DH)
        return pltpu.make_async_copy(wq_hbm.at[:, cols], wql_v.at[ci], wql_sem.at[ci])

    def wot_cp():
        return pltpu.make_async_copy(wot_hbm, wot_v, w_sem.at[0])

    def wqx_cp():
        return pltpu.make_async_copy(wq_hbm.at[:, pl.ds(HXO * DH, HX * DH)], wqx_v, w_sem.at[1])

    def k_cp(g):
        bs = pl.ds(g * GB, GB)
        return pltpu.make_async_copy(k_hbm.at[bs], k_v.at[bs], kv_sem.at[2 * g])

    def v_cp(g):
        bs = pl.ds(g * GB, GB)
        return pltpu.make_async_copy(v_hbm.at[bs], v_v.at[bs], kv_sem.at[2 * g + 1])

    def out_cp(g, p):
        rows = pl.ds(aligned(g * GM + PIECES[p], 16), PIECES[p + 1] - PIECES[p])
        return pltpu.make_async_copy(y_v.at[rows], out_hbm.at[rows], out_sem.at[g * NP + p])

    def start_range(cp, lo, hi, prio):
        if hi - lo == 1:
            cp(lo).start(priority=prio)
        elif hi > lo:
            def body(i, carry):
                cp(i).start(priority=prio)
                return carry
            jax.lax.fori_loop(lo, hi, body, 0)

    px, ph = 0, 0
    for si, (nx, nh) in enumerate(STAGES):
        prio = 0 if si == 0 else 1
        start_range(wq0_cp, ph, nh, prio)
        start_range(x_cp, px, nx, prio)
        px, ph = nx, nh
    start_range(wql_cp, 0, NL, 1)
    k_cp(0).start(priority=1)
    v_cp(0).start(priority=1)
    wot_cp().start(priority=1)
    wqx_cp().start(priority=1)

    def start_kv(g, carry):
        k_cp(g).start(priority=1)
        v_cp(g).start(priority=1)
        return carry

    jax.lax.fori_loop(1, NG, start_kv, 0)
    o_v[GM:GM + 16, 0:128] = jnp.zeros((16, 128), bf16)

    def project(xs, w):
        q = jnp.dot(xs, w, preferred_element_type=f32)
        return (q * Q_SCALE).astype(bf16)

    def startup_piece(x0, x1, h0, h1):
        if x1 > x0 and h1 > h0:
            ns = 4 // math.gcd(4, h1 - h0)
            rs = (x1 - x0) * XR // ns
            for j in range(ns):
                r0 = x0 * XR + j * rs
                q0_v[r0:r0 + rs, h0 * DH:h1 * DH] = project(
                    x_v[r0:r0 + rs, :], wq0_v[:, h0 * DH:h1 * DH])

    def startup():
        px, ph = 0, 0
        for nx, nh in STAGES:
            for h in range(ph, nh):
                wq0_cp(h).wait()
            for i in range(px, nx):
                x_cp(i).wait()
            startup_piece(0, px, ph, nh)
            startup_piece(px, nx, 0, nh)
            px, ph = nx, nh

    def projection_block(ci):
        wql_cp(ci).wait()
        ql_v[ci] = project(x_v[...], wql_v[ci])

    def attention_block(g):
        @pl.when(g == 0)
        def _():
            wot_cp().wait()
            wqx_cp().wait()

        k_cp(g).wait()
        v_cp(g).wait()
        row0 = pl.multiple_of(g * GM, GM)
        zero_row = pl.multiple_of(GM + jnp.minimum(g, 0) * 16, 16)

        def q_head(hq, bb):
            rows = pl.ds(row0 + bb * SQ, SQ)
            if hq < H0:
                return q0_v[rows, hq * DH:(hq + 1) * DH]
            if hq >= HXO:
                return qx_v[bb * SQ:(bb + 1) * SQ, (hq - HXO) * DH:(hq - HXO + 1) * DH]
            ci, off = divmod(hq - H0, HL)
            return ql_v[ci, rows, off * DH:(off + 1) * DH]

        def scores(bb, h):
            q = jnp.concatenate([q_head(REP * h + r, bb) for r in range(REP)], axis=0)
            return jax.lax.dot_general(q, k_v[g * GB + bb, h], NT_DIMS, preferred_element_type=f32)

        def softmax_pv(bb, h, s):
            m = jnp.max(s, axis=-1, keepdims=True)
            p = jnp.exp2(s - m)
            l = jnp.sum(p, axis=-1, keepdims=True)
            o = jnp.dot(p.astype(bf16), v_v[g * GB + bb, h], preferred_element_type=f32)
            o = (o * pl.reciprocal(l, approx=True)).astype(bf16)
            for r in range(REP):
                col = (REP * h + r) * DH
                o_v[bb * SQ:(bb + 1) * SQ, col:col + DH] = o[r * SQ:(r + 1) * SQ]

        def out_rest(t):
            r = jax.lax.dot_general(wot_v[DF:D, :], o_v[t * TT:(t + 1) * TT, :], NT_DIMS,
                                    preferred_element_type=f32)
            y_v[pl.ds(row0 + t * TT, TT), DF:D] = r.T.astype(bf16)

        def out_full(p, w, zero):
            lo, hi = PIECES[p], PIECES[p + 1]
            a = o_v[lo:hi, :]
            if zero is not None:
                tile = (a[0:16, 0:128].astype(f32) + zero).astype(bf16)
                a = jnp.concatenate(
                    [jnp.concatenate([tile, a[0:16, 128:]], axis=1), a[16:]], axis=0)
            r = jax.lax.dot_general(a, wot_v[w * 128:(w + 1) * 128, :], NT_DIMS,
                                    preferred_element_type=f32)
            y_v[pl.ds(row0 + lo, hi - lo), w * 128:(w + 1) * 128] = r.astype(bf16)

        qx_v[...] = project(x_v[pl.ds(row0, GM), :], wqx_v[...])

        units = [(bb, h) for bb in range(GB) for h in range(HKV)]
        zeros = {}
        s = scores(*units[0])
        for i, u in enumerate(units):
            if i + 1 < len(units):
                s_next = scores(*units[i + 1])
            else:
                out_rest(0)
            if i in zeros:
                top = jnp.concatenate([s[0:8, 0:128] + zeros.pop(i), s[0:8, 128:]], axis=1)
                s = jnp.concatenate([top, s[8:]], axis=0)
            softmax_pv(*u, s)
            if i + O_LAG < len(units):
                zeros[i + O_LAG] = o_v[pl.ds(zero_row, 16), 0:128].astype(f32)[0:8]
            s = s_next

        out_rest(1)
        jobs = [(p, w) for p in range(NP) for w in range(NW)]
        zeros = {}
        for j, (p, w) in enumerate(jobs):
            out_full(p, w, zeros.pop(j, None))
            if j == 0:
                out_rest(2)
            if w == NW - 1:
                out_cp(g, p).start()
                if j + OUT_LAG < len(jobs):
                    y_v[M:M + 16, 0:128] = jnp.zeros((16, 128), bf16)
                    zeros[j + OUT_LAG] = y_v[M:M + 16, 0:128].astype(f32)

    def step(it, carry):
        @pl.when(it == 0)
        def _():
            startup()

        @pl.when(jnp.logical_and(it >= 1, it <= NL))
        def _():
            projection_block(it - 1)

        @pl.when(it > NL)
        def _():
            attention_block(it - NL - 1)

        return carry

    jax.lax.fori_loop(0, 1 + NL + NG, step, 0)
    for g in range(NG):
        for p in range(NP):
            out_cp(g, p).wait()


@jax.jit
def pallas_standalone__gqa_block_cached__near_ridge_kernel(
    x: jax.Array,
    k_cache: jax.Array,
    v_cache: jax.Array,
    wq: jax.Array,
    wo: jax.Array,
):
    assert x.shape == (B, SQ, D) and k_cache.shape == (B, HKV, SK, DH) == v_cache.shape
    assert wq.shape == (D, HQ * DH) and wo.shape == (HQ * DH, D)
    hbm = pl.BlockSpec(memory_space=pl.ANY)
    out = pl.pallas_call(
        _kernel,
        in_specs=[hbm] * 5,
        out_specs=hbm,
        out_shape=jax.ShapeDtypeStruct((M, D), x.dtype),
        scratch_shapes=[
            pltpu.VMEM((M, D), bf16),
            pltpu.VMEM((D, H0 * DH), bf16),
            pltpu.VMEM((NL, D, HL * DH), bf16),
            pltpu.VMEM((D, HX * DH), bf16),
            pltpu.VMEM((D, HQ * DH), bf16),
            pltpu.VMEM((B, HKV, SK, DH), bf16),
            pltpu.VMEM((B, HKV, SK, DH), bf16),
            pltpu.VMEM((M, H0 * DH), bf16),
            pltpu.VMEM((NL, M, HL * DH), bf16),
            pltpu.VMEM((GM, HX * DH), bf16),
            pltpu.VMEM((GM + 16, HQ * DH), bf16),
            pltpu.VMEM((M + 16, D), bf16),
            pltpu.SemaphoreType.DMA((NX,)),
            pltpu.SemaphoreType.DMA((H0,)),
            pltpu.SemaphoreType.DMA((NL,)),
            pltpu.SemaphoreType.DMA((2,)),
            pltpu.SemaphoreType.DMA((2 * NG,)),
            pltpu.SemaphoreType.DMA((NP * NG,)),
        ],
        compiler_params=pltpu.CompilerParams(
            vmem_limit_bytes=120 * 1024 * 1024,
            disable_semaphore_checks=True,
            disable_bounds_checks=True,
        ),
    )(x.reshape(M, D), k_cache, v_cache, wq, wo.T)
    return out.reshape(B, SQ, D)
```

```python
import math

import jax
import jax.numpy as jnp
import jax.experimental.pallas as pl
import jax.experimental.pallas.tpu as pltpu

B, SQ, D = 16, 96, 576
HQ, HKV, SK, DH = 32, 16, 512, 128
REP = HQ // HKV
M = B * SQ
GB = 4
NG = B // GB
GM = GB * SQ
TT = 128
DF = (D // 128) * 128
XR = 128
NX = M // XR

H0 = 4
HL = 12
NL = 2
HX = 4
HXO = HQ - HX
assert H0 + NL * HL + HX == HQ

STAGES = ((1, 2), (2, 3), (3, 4), (6, 4), (NX, H0))
PIECES = (0, 320, 384)
NP = len(PIECES) - 1
NW = DF // 128
SPLIT = 256
OUT_COPIES = tuple((p, 0, D) for p in range(NP - 1)) + ((NP - 1, SPLIT, D), (NP - 1, 0, SPLIT))
O_LAG = 3
OUT_LAG = 3

NT_DIMS = (((1,), (1,)), ((), ()))
Q_SCALE = (DH ** -0.5) * math.log2(math.e)
bf16 = jnp.bfloat16
f32 = jnp.float32


def _kernel(x_hbm, k_hbm, v_hbm, wq_hbm, wot_hbm, out_hbm,
            x_v, wq0_v, wql_v, wqx_v, wot_v, k_v, v_v, q0_v, ql_v, qx_v, o_v, y_v,
            x_sem, wq0_sem, wql_sem, w_sem, kv_sem, out_sem):
    def aligned(i, n):
        return i if isinstance(i, int) else pl.multiple_of(i, n)

    def x_cp(i):
        rows = pl.ds(aligned(i * XR, XR), XR)
        return pltpu.make_async_copy(x_hbm.at[rows], x_v.at[rows], x_sem.at[i])

    def wq0_cp(h):
        cols = pl.ds(aligned(h * DH, DH), DH)
        return pltpu.make_async_copy(wq_hbm.at[:, cols], wq0_v.at[:, cols], wq0_sem.at[h])

    def wql_cp(ci):
        cols = pl.ds(aligned((H0 + ci * HL) * DH, DH), HL * DH)
        return pltpu.make_async_copy(wq_hbm.at[:, cols], wql_v.at[ci], wql_sem.at[ci])

    def wot_cp():
        return pltpu.make_async_copy(wot_hbm, wot_v, w_sem.at[0])

    def wqx_cp():
        return pltpu.make_async_copy(wq_hbm.at[:, pl.ds(HXO * DH, HX * DH)], wqx_v, w_sem.at[1])

    def k_cp(g):
        bs = pl.ds(g * GB, GB)
        return pltpu.make_async_copy(k_hbm.at[bs], k_v.at[bs], kv_sem.at[2 * g])

    def v_cp(g):
        bs = pl.ds(g * GB, GB)
        return pltpu.make_async_copy(v_hbm.at[bs], v_v.at[bs], kv_sem.at[2 * g + 1])

    def out_cp(g, n):
        p, c0, c1 = OUT_COPIES[n]
        rows = pl.ds(aligned(g * GM + PIECES[p], 16), PIECES[p + 1] - PIECES[p])
        cols = pl.ds(c0, c1 - c0)
        return pltpu.make_async_copy(y_v.at[rows, cols], out_hbm.at[rows, cols],
                                     out_sem.at[g * len(OUT_COPIES) + n])

    def start_range(cp, lo, hi, prio):
        if hi - lo == 1:
            cp(lo).start(priority=prio)
        elif hi > lo:
            def body(i, carry):
                cp(i).start(priority=prio)
                return carry
            jax.lax.fori_loop(lo, hi, body, 0)

    px, ph = 0, 0
    for si, (nx, nh) in enumerate(STAGES):
        prio = 0 if si == 0 else 1
        start_range(wq0_cp, ph, nh, prio)
        start_range(x_cp, px, nx, prio)
        px, ph = nx, nh
    start_range(wql_cp, 0, NL, 1)
    k_cp(0).start(priority=1)
    v_cp(0).start(priority=1)
    wot_cp().start(priority=1)
    wqx_cp().start(priority=1)

    def start_kv(g, carry):
        k_cp(g).start(priority=1)
        v_cp(g).start(priority=1)
        return carry

    jax.lax.fori_loop(1, NG, start_kv, 0)
    o_v[GM:GM + 16, 0:128] = jnp.zeros((16, 128), bf16)

    def project(xs, w):
        q = jnp.dot(xs, w, preferred_element_type=f32)
        return (q * Q_SCALE).astype(bf16)

    def startup_piece(x0, x1, h0, h1):
        if x1 > x0 and h1 > h0:
            ns = 4 // math.gcd(4, h1 - h0)
            rs = (x1 - x0) * XR // ns
            for j in range(ns):
                r0 = x0 * XR + j * rs
                q0_v[r0:r0 + rs, h0 * DH:h1 * DH] = project(
                    x_v[r0:r0 + rs, :], wq0_v[:, h0 * DH:h1 * DH])

    def startup():
        px, ph = 0, 0
        for nx, nh in STAGES:
            for h in range(ph, nh):
                wq0_cp(h).wait()
            for i in range(px, nx):
                x_cp(i).wait()
            startup_piece(0, px, ph, nh)
            startup_piece(px, nx, 0, nh)
            px, ph = nx, nh

    def projection_block(ci):
        wql_cp(ci).wait()
        ql_v[ci] = project(x_v[...], wql_v[ci])

    def attention_block(g):
        @pl.when(g == 0)
        def _():
            wot_cp().wait()
            wqx_cp().wait()

        k_cp(g).wait()
        v_cp(g).wait()
        row0 = pl.multiple_of(g * GM, GM)
        zero_row = pl.multiple_of(GM + jnp.minimum(g, 0) * 16, 16)

        def q_head(hq, bb):
            rows = pl.ds(row0 + bb * SQ, SQ)
            if hq < H0:
                return q0_v[rows, hq * DH:(hq + 1) * DH]
            if hq >= HXO:
                return qx_v[bb * SQ:(bb + 1) * SQ, (hq - HXO) * DH:(hq - HXO + 1) * DH]
            ci, off = divmod(hq - H0, HL)
            return ql_v[ci, rows, off * DH:(off + 1) * DH]

        def scores(bb, h):
            q = jnp.concatenate([q_head(REP * h + r, bb) for r in range(REP)], axis=0)
            return jax.lax.dot_general(q, k_v[g * GB + bb, h], NT_DIMS, preferred_element_type=f32)

        def softmax_pv(bb, h, s):
            m = jnp.max(s, axis=-1, keepdims=True)
            p = jnp.exp2(s - m)
            l = jnp.sum(p, axis=-1, keepdims=True)
            o = jnp.dot(p.astype(bf16), v_v[g * GB + bb, h], preferred_element_type=f32)
            o = (o * pl.reciprocal(l, approx=True)).astype(bf16)
            for r in range(REP):
                col = (REP * h + r) * DH
                o_v[bb * SQ:(bb + 1) * SQ, col:col + DH] = o[r * SQ:(r + 1) * SQ]

        def out_rest(t):
            r = jax.lax.dot_general(wot_v[DF:D, :], o_v[t * TT:(t + 1) * TT, :], NT_DIMS,
                                    preferred_element_type=f32)
            y_v[pl.ds(row0 + t * TT, TT), DF:D] = r.T.astype(bf16)

        def out_full(p, w, zero):
            lo, hi = PIECES[p], PIECES[p + 1]
            a = o_v[lo:hi, :]
            if zero is not None:
                tile = (a[0:16, 0:128].astype(f32) + zero).astype(bf16)
                a = jnp.concatenate(
                    [jnp.concatenate([tile, a[0:16, 128:]], axis=1), a[16:]], axis=0)
            r = jax.lax.dot_general(a, wot_v[w * 128:(w + 1) * 128, :], NT_DIMS,
                                    preferred_element_type=f32)
            y_v[pl.ds(row0 + lo, hi - lo), w * 128:(w + 1) * 128] = r.astype(bf16)

        qx_v[...] = project(x_v[pl.ds(row0, GM), :], wqx_v[...])

        units = [(bb, h) for bb in range(GB) for h in range(HKV)]
        zeros = {}
        s = scores(*units[0])
        for i, u in enumerate(units):
            if i + 1 < len(units):
                s_next = scores(*units[i + 1])
            else:
                out_rest(0)
            if i in zeros:
                top = jnp.concatenate([s[0:8, 0:128] + zeros.pop(i), s[0:8, 128:]], axis=1)
                s = jnp.concatenate([top, s[8:]], axis=0)
            softmax_pv(*u, s)
            if i + O_LAG < len(units):
                zeros[i + O_LAG] = o_v[pl.ds(zero_row, 16), 0:128].astype(f32)[0:8]
            s = s_next

        out_rest(1)
        jobs = [(p, w) for p in range(NP) for w in reversed(range(NW))]
        zeros = {}
        for j, (p, w) in enumerate(jobs):
            out_full(p, w, zeros.pop(j, None))
            if j == 0:
                out_rest(2)
            for n, (cp, c0, _) in enumerate(OUT_COPIES):
                if (cp, c0) == (p, w * 128):
                    out_cp(g, n).start()
                    lag = min(OUT_LAG, len(jobs) - 1 - j)
                    if lag >= 2 and j + lag not in zeros:
                        y_v[M:M + 16, 0:128] = jnp.zeros((16, 128), bf16)
                        zeros[j + lag] = y_v[M:M + 16, 0:128].astype(f32)

    def step(it, carry):
        @pl.when(it == 0)
        def _():
            startup()

        @pl.when(jnp.logical_and(it >= 1, it <= NL))
        def _():
            projection_block(it - 1)

        @pl.when(it > NL)
        def _():
            attention_block(it - NL - 1)

        return carry

    jax.lax.fori_loop(0, 1 + NL + NG, step, 0)
    for g in range(NG):
        for n in range(len(OUT_COPIES)):
            out_cp(g, n).wait()


@jax.jit
def pallas_standalone__gqa_block_cached__near_ridge_kernel(
    x: jax.Array,
    k_cache: jax.Array,
    v_cache: jax.Array,
    wq: jax.Array,
    wo: jax.Array,
):
    assert x.shape == (B, SQ, D) and k_cache.shape == (B, HKV, SK, DH) == v_cache.shape
    assert wq.shape == (D, HQ * DH) and wo.shape == (HQ * DH, D)
    hbm = pl.BlockSpec(memory_space=pl.ANY)
    out = pl.pallas_call(
        _kernel,
        in_specs=[hbm] * 5,
        out_specs=hbm,
        out_shape=jax.ShapeDtypeStruct((M, D), x.dtype),
        scratch_shapes=[
            pltpu.VMEM((M, D), bf16),
            pltpu.VMEM((D, H0 * DH), bf16),
            pltpu.VMEM((NL, D, HL * DH), bf16),
            pltpu.VMEM((D, HX * DH), bf16),
            pltpu.VMEM((D, HQ * DH), bf16),
            pltpu.VMEM((B, HKV, SK, DH), bf16),
            pltpu.VMEM((B, HKV, SK, DH), bf16),
            pltpu.VMEM((M, H0 * DH), bf16),
            pltpu.VMEM((NL, M, HL * DH), bf16),
            pltpu.VMEM((GM, HX * DH), bf16),
            pltpu.VMEM((GM + 16, HQ * DH), bf16),
            pltpu.VMEM((M + 16, D), bf16),
            pltpu.SemaphoreType.DMA((NX,)),
            pltpu.SemaphoreType.DMA((H0,)),
            pltpu.SemaphoreType.DMA((NL,)),
            pltpu.SemaphoreType.DMA((2,)),
            pltpu.SemaphoreType.DMA((2 * NG,)),
            pltpu.SemaphoreType.DMA((len(OUT_COPIES) * NG,)),
        ],
        compiler_params=pltpu.CompilerParams(
            vmem_limit_bytes=120 * 1024 * 1024,
            disable_semaphore_checks=True,
            disable_bounds_checks=True,
        ),
    )(x.reshape(M, D), k_cache, v_cache, wq, wo.T)
    return out.reshape(B, SQ, D)
```

```python
import math

import jax
import jax.numpy as jnp
import jax.experimental.pallas as pl
import jax.experimental.pallas.tpu as pltpu

B, SQ, D = 16, 96, 576
HQ, HKV, SK, DH = 32, 16, 512, 128
REP = HQ // HKV
M = B * SQ
GB = 4
NG = B // GB
GM = GB * SQ
TT = 128
DF = (D // 128) * 128
XR = 128
NX = M // XR

H0 = 4
HL = 12
NL = 2
HX = 4
HXO = HQ - HX
assert H0 + NL * HL + HX == HQ

STAGES = ((1, 2), (2, 3), (3, 4), (6, 4), (NX, H0))
PIECES = (0, 320, 384)
NP = len(PIECES) - 1
NW = DF // 128
O_LAG = 3
OUT_LAG = 3

NT_DIMS = (((1,), (1,)), ((), ()))
Q_SCALE = (DH ** -0.5) * math.log2(math.e)
bf16 = jnp.bfloat16
f32 = jnp.float32


def _kernel(x_hbm, k_hbm, v_hbm, wq_hbm, wot_hbm, out_hbm,
            x_v, wq0_v, wql_v, wqx_v, wot_v, k_v, v_v, q0_v, ql_v, qx_v, o_v, y_v,
            x_sem, wq0_sem, wql_sem, w_sem, kv_sem, out_sem):
    def aligned(i, n):
        return i if isinstance(i, int) else pl.multiple_of(i, n)

    def x_cp(i):
        rows = pl.ds(aligned(i * XR, XR), XR)
        return pltpu.make_async_copy(x_hbm.at[rows], x_v.at[rows], x_sem.at[i])

    def wq0_cp(h):
        cols = pl.ds(aligned(h * DH, DH), DH)
        return pltpu.make_async_copy(wq_hbm.at[:, cols], wq0_v.at[:, cols], wq0_sem.at[h])

    def wql_cp(ci):
        cols = pl.ds(aligned((H0 + ci * HL) * DH, DH), HL * DH)
        return pltpu.make_async_copy(wq_hbm.at[:, cols], wql_v.at[ci], wql_sem.at[ci])

    def wot_cp():
        return pltpu.make_async_copy(wot_hbm, wot_v, w_sem.at[0])

    def wqx_cp():
        return pltpu.make_async_copy(wq_hbm.at[:, pl.ds(HXO * DH, HX * DH)], wqx_v, w_sem.at[1])

    def k_cp(g):
        bs = pl.ds(g * GB, GB)
        return pltpu.make_async_copy(k_hbm.at[bs], k_v.at[bs], kv_sem.at[2 * g])

    def v_cp(g):
        bs = pl.ds(g * GB, GB)
        return pltpu.make_async_copy(v_hbm.at[bs], v_v.at[bs], kv_sem.at[2 * g + 1])

    def out_cp(g, p):
        rows = pl.ds(aligned(g * GM + PIECES[p], 16), PIECES[p + 1] - PIECES[p])
        return pltpu.make_async_copy(y_v.at[rows], out_hbm.at[rows], out_sem.at[g * NP + p])

    def start_range(cp, lo, hi, prio):
        if hi - lo == 1:
            cp(lo).start(priority=prio)
        elif hi > lo:
            def body(i, carry):
                cp(i).start(priority=prio)
                return carry
            jax.lax.fori_loop(lo, hi, body, 0)

    px, ph = 0, 0
    for si, (nx, nh) in enumerate(STAGES):
        prio = 0 if si == 0 else 1
        start_range(wq0_cp, ph, nh, prio)
        start_range(x_cp, px, nx, prio)
        px, ph = nx, nh
    start_range(wql_cp, 0, NL, 1)
    k_cp(0).start(priority=1)
    v_cp(0).start(priority=1)
    wot_cp().start(priority=1)
    wqx_cp().start(priority=1)

    def start_kv(g, carry):
        k_cp(g).start(priority=1)
        v_cp(g).start(priority=1)
        return carry

    jax.lax.fori_loop(1, NG, start_kv, 0)
    o_v[GM:GM + 16, 0:128] = jnp.zeros((16, 128), bf16)

    def project(xs, w):
        q = jnp.dot(xs, w, preferred_element_type=f32)
        return (q * Q_SCALE).astype(bf16)

    def startup_piece(x0, x1, h0, h1):
        if x1 > x0 and h1 > h0:
            ns = 4 // math.gcd(4, h1 - h0)
            rs = (x1 - x0) * XR // ns
            for j in range(ns):
                r0 = x0 * XR + j * rs
                q0_v[r0:r0 + rs, h0 * DH:h1 * DH] = project(
                    x_v[r0:r0 + rs, :], wq0_v[:, h0 * DH:h1 * DH])

    def startup():
        px, ph = 0, 0
        for nx, nh in STAGES:
            for h in range(ph, nh):
                wq0_cp(h).wait()
            for i in range(px, nx):
                x_cp(i).wait()
            startup_piece(0, px, ph, nh)
            startup_piece(px, nx, 0, nh)
            px, ph = nx, nh

    def projection_block(ci):
        wql_cp(ci).wait()
        ql_v[ci] = project(x_v[...], wql_v[ci])

    def attention_block(g):
        @pl.when(g == 0)
        def _():
            wot_cp().wait()
            wqx_cp().wait()

        k_cp(g).wait()
        v_cp(g).wait()
        row0 = pl.multiple_of(g * GM, GM)
        zero_row = pl.multiple_of(GM + jnp.minimum(g, 0) * 16, 16)

        def q_head(hq, bb):
            rows = pl.ds(row0 + bb * SQ, SQ)
            if hq < H0:
                return q0_v[rows, hq * DH:(hq + 1) * DH]
            if hq >= HXO:
                return qx_v[bb * SQ:(bb + 1) * SQ, (hq - HXO) * DH:(hq - HXO + 1) * DH]
            ci, off = divmod(hq - H0, HL)
            return ql_v[ci, rows, off * DH:(off + 1) * DH]

        def scores(bb, h):
            q = jnp.concatenate([q_head(REP * h + r, bb) for r in range(REP)], axis=0)
            return jax.lax.dot_general(q, k_v[g * GB + bb, h], NT_DIMS, preferred_element_type=f32)

        def softmax_pv(bb, h, s):
            m = jnp.max(s, axis=-1, keepdims=True)
            p = jnp.exp2(s - m)
            l = jnp.sum(p, axis=-1, keepdims=True)
            o = jnp.dot(p.astype(bf16), v_v[g * GB + bb, h], preferred_element_type=f32)
            o = (o * pl.reciprocal(l, approx=True)).astype(bf16)
            for r in range(REP):
                col = (REP * h + r) * DH
                o_v[bb * SQ:(bb + 1) * SQ, col:col + DH] = o[r * SQ:(r + 1) * SQ]

        def out_rest(t):
            r = jax.lax.dot_general(wot_v[DF:D, :], o_v[t * TT:(t + 1) * TT, :], NT_DIMS,
                                    preferred_element_type=f32)
            y_v[pl.ds(row0 + t * TT, TT), DF:D] = r.T.astype(bf16)

        def out_full(p, w, zero):
            lo, hi = PIECES[p], PIECES[p + 1]
            a = o_v[lo:hi, :]
            if zero is not None:
                tile = (a[0:16, 0:128].astype(f32) + zero).astype(bf16)
                a = jnp.concatenate(
                    [jnp.concatenate([tile, a[0:16, 128:]], axis=1), a[16:]], axis=0)
            r = jax.lax.dot_general(a, wot_v[w * 128:(w + 1) * 128, :], NT_DIMS,
                                    preferred_element_type=f32)
            y_v[pl.ds(row0 + lo, hi - lo), w * 128:(w + 1) * 128] = r.astype(bf16)

        qx_v[...] = project(x_v[pl.ds(row0, GM), :], wqx_v[...])

        units = [(bb, h) for bb in range(GB) for h in range(HKV)]
        zeros = {}
        s = scores(*units[0])
        for i, u in enumerate(units):
            if i + 1 < len(units):
                s_next = scores(*units[i + 1])
            else:
                out_rest(0)
            if i in zeros:
                top = jnp.concatenate([s[0:8, 0:128] + zeros.pop(i), s[0:8, 128:]], axis=1)
                s = jnp.concatenate([top, s[8:]], axis=0)
            softmax_pv(*u, s)
            if i + O_LAG < len(units):
                zeros[i + O_LAG] = o_v[pl.ds(zero_row, 16), 0:128].astype(f32)[0:8]
            s = s_next

        out_rest(1)
        jobs = [(p, w) for p in range(NP) for w in range(NW)]
        zeros = {}
        for j, (p, w) in enumerate(jobs):
            out_full(p, w, zeros.pop(j, None))
            if j == 0:
                out_rest(2)
            if w == NW - 1:
                out_cp(g, p).start()
                if j + OUT_LAG < len(jobs):
                    y_v[M:M + 16, 0:128] = jnp.zeros((16, 128), bf16)
                    zeros[j + OUT_LAG] = y_v[M:M + 16, 0:128].astype(f32)

    def step(it, carry):
        @pl.when(it == 0)
        def _():
            startup()

        @pl.when(jnp.logical_and(it >= 1, it <= NL))
        def _():
            projection_block(it - 1)

        @pl.when(it > NL)
        def _():
            attention_block(it - NL - 1)

        return carry

    jax.lax.fori_loop(0, 1 + NL + NG, step, 0)
    for g in range(NG):
        for p in range(NP):
            out_cp(g, p).wait()


@jax.jit
def pallas_standalone__gqa_block_cached__near_ridge_kernel(
    x: jax.Array,
    k_cache: jax.Array,
    v_cache: jax.Array,
    wq: jax.Array,
    wo: jax.Array,
):
    assert x.shape == (B, SQ, D) and k_cache.shape == (B, HKV, SK, DH) == v_cache.shape
    assert wq.shape == (D, HQ * DH) and wo.shape == (HQ * DH, D)
    hbm = pl.BlockSpec(memory_space=pl.ANY)
    out = pl.pallas_call(
        _kernel,
        in_specs=[hbm] * 5,
        out_specs=hbm,
        out_shape=jax.ShapeDtypeStruct((M, D), x.dtype),
        scratch_shapes=[
            pltpu.VMEM((M, D), bf16),
            pltpu.VMEM((D, H0 * DH), bf16),
            pltpu.VMEM((NL, D, HL * DH), bf16),
            pltpu.VMEM((D, HX * DH), bf16),
            pltpu.VMEM((D, HQ * DH), bf16),
            pltpu.VMEM((B, HKV, SK, DH), bf16),
            pltpu.VMEM((B, HKV, SK, DH), bf16),
            pltpu.VMEM((M, H0 * DH), bf16),
            pltpu.VMEM((NL, M, HL * DH), bf16),
            pltpu.VMEM((GM, HX * DH), bf16),
            pltpu.VMEM((GM + 16, HQ * DH), bf16),
            pltpu.VMEM((M + 16, D), bf16),
            pltpu.SemaphoreType.DMA((NX,)),
            pltpu.SemaphoreType.DMA((H0,)),
            pltpu.SemaphoreType.DMA((NL,)),
            pltpu.SemaphoreType.DMA((2,)),
            pltpu.SemaphoreType.DMA((2 * NG,)),
            pltpu.SemaphoreType.DMA((NP * NG,)),
        ],
        compiler_params=pltpu.CompilerParams(
            vmem_limit_bytes=120 * 1024 * 1024,
            disable_semaphore_checks=True,
            disable_bounds_checks=True,
        ),
    )(x.reshape(M, D), k_cache, v_cache, wq, wo.T)
    return out.reshape(B, SQ, D)
```
